```python
import os as _os
_os.environ.setdefault("JAX_PLATFORMS", "cpu")
import jax
import jax.numpy as jnp

def _softmax(x, axis=-1):
    return jax.nn.softmax(x, axis=axis)
def _gelu(x):
    return jax.nn.gelu(x, approximate=True)
def _silu(x):
    return jax.nn.silu(x)
def _sigmoid(x):
    return jax.nn.sigmoid(x)
def _layernorm(x, axis=-1, eps=1e-5):
    m = jnp.mean(x, axis=axis, keepdims=True)
    v = jnp.var(x, axis=axis, keepdims=True)
    return (x - m) / jnp.sqrt(v + eps)
def _scatter_add(tgt, idx, src, axis=0):
    return tgt.at[idx].add(src)
def _segment_sum(src, seg, n):
    return jax.ops.segment_sum(src, seg, n)
class _Rng:
    def __init__(self, key):
        self._k = key
    def _next(self):
        self._k, sub = jax.random.split(self._k)
        return sub
    def normal(self, shape):
        return jax.random.normal(self._next(), shape, dtype=jnp.bfloat16)
    def randint(self, lo, hi, shape):
        return jax.random.randint(self._next(), shape, lo, hi, dtype=jnp.int32)
    def uniform(self, shape, lo=0.0, hi=1.0):
        return jax.random.uniform(self._next(), shape, jnp.bfloat16, lo, hi)
    def permutation(self, n):
        return jax.random.permutation(self._next(), n)


kernel_name = 'gated_mix__linear_attn_block__glu_gated_swiglu__prompt'

def setup_inputs():
    _rng = _Rng(jax.random.key(int.from_bytes(__import__("os").urandom(4), "little")))
    _w = (lambda a: (lambda t: t.astype(jnp.bfloat16) if jnp.issubdtype(t.dtype, jnp.floating) else t)(jnp.asarray(a)))
    def _A_setup():
        B, S, D = 1, 2048, 1024
        return {
            "x": _w((lambda *s: _rng.normal(s) * 0.05)(B, S, D)),
            "wqkv": _w((lambda *s: _rng.normal(s) * 0.8)(D, 3 * D)),
            "wo": _w((lambda *s: _rng.normal(s) * 0.05)(D, D)),
        }
    _A_in = _A_setup()

    def _B_setup():
        B, S, D, F = 1, 2048, 1024, 3584
        return {
            "x": _w((lambda *s: _rng.normal(s) * 0.05)(B, S, D)),
            "w1": _w((lambda *s: _rng.normal(s) * 1.6)(D, F) * (2.0 / D) ** 0.5),
            "w3": _w((lambda *s: _rng.normal(s) * 1.6)(D, F) * (2.0 / D) ** 0.5),
            "w2": _w((lambda *s: _rng.normal(s) * 1.6)(F, D) * (2.0 / F) ** 0.5),
        }
    _B_in = _B_setup()

    return {
        "A_x": _A_in["x"],
        "A_wqkv": _A_in["wqkv"],
        "A_wo": _A_in["wo"],
        "B_x": _B_in["x"],
        "B_w1": _B_in["w1"],
        "B_w3": _B_in["w3"],
        "B_w2": _B_in["w2"],
        "gate_w": _w((lambda *s: _rng.normal(s) * 0.05)(1024) * 16.0),
    }

def reference(A_x, A_wqkv, A_wo, B_x, B_w1, B_w3, B_w2, gate_w):
    def _A_ref(x, wqkv, wo):
        B, S, D = x.shape
        H = 32; Dh = D // H
        qkv = (lambda x, *d: x.transpose(*d))((x @ wqkv).reshape(B, S, 3, H, Dh), 2, 0, 3, 1, 4)
        q, k, v = qkv[0], qkv[1], qkv[2]
        phi = lambda t: jnp.where(t > 0, t + 1, jnp.exp(t)) + 1e-6
        pq, pk = phi(q), phi(k)
        kv = jnp.einsum("bhsd,bhse->bhde", pk, v)
        z = jnp.einsum("bhsd->bhd", pk)
        num = jnp.einsum("bhqd,bhde->bhqe", pq, kv)
        den = jnp.einsum("bhqd,bhd->bhq", pq, z)[..., None] + 1e-6
        o = num / den
        return (lambda x, *d: x.transpose(*d))(o, 0, 2, 1, 3).reshape(B, S, D) @ wo

    def _B_ref(x, w1, w3, w2):
        gate = jnp.einsum("bsd,df->bsf", x, w1)
        up = jnp.einsum("bsd,df->bsf", x, w3)
        h = _silu(gate) * up
        out = jnp.einsum("bsf,fd->bsd", h, w2)
        return out

    x = A_x
    g = _sigmoid((x * gate_w).sum(-1, keepdims=True))
    a = _A_ref(x, A_wqkv, A_wo)
    b = _B_ref(x, B_w1, B_w3, B_w2)
    return g * a + (1 - g) * b
```

```python
import jax
import jax.numpy as jnp
from jax import lax
import jax.experimental.pallas as pl
import jax.experimental.pallas.tpu as pltpu

_F32, _BF16 = jnp.float32, jnp.bfloat16
_NT = (((1,), (1,)), ((), ()))
_TN = (((0,), (0,)), ((), ()))
_HEAD = 32


def _phi(t):
    return jnp.where(t > 0, t + 1.0, jnp.exp(t)) + 1e-6


def _recip(d):
    r = pl.reciprocal(d, approx=True)
    return r * (2.0 - d * r)


@jax.jit
def pallas_gated_mix__linear_attn_block__glu_gated_swiglu__prompt_kernel(
    A_x, A_wqkv, A_wo, B_x, B_w1, B_w3, B_w2, gate_w,
):
    del B_x
    B, S, D = A_x.shape
    F = B_w1.shape[1]
    TM, TK, FC = 256, 256, 512
    NT, NK, NF, NG = S // TM, S // TK, F // FC, D // 128
    assert B == 1

    def kernel(x_hbm, wqkv_hbm, wo_hbm, w1_hbm, w3_hbm, w2_hbm, gw_ref, o_hbm,
               x_v, wq_v, wk_v, wv_v, wo_v, w1_v, w3_v, w2_v, T_v, z_v, M_v, zb_v, ob_v,
               sx, sw, sf, so):
        def cx(i):
            r = pl.ds(i * TK, TK)
            return pltpu.make_async_copy(x_hbm.at[r], x_v.at[r], sx.at[i])
        cq = pltpu.make_async_copy(wqkv_hbm.at[:, pl.ds(0, D)], wq_v, sw.at[0])
        ck = pltpu.make_async_copy(wqkv_hbm.at[:, pl.ds(D, D)], wk_v, sw.at[1])
        cv = pltpu.make_async_copy(wqkv_hbm.at[:, pl.ds(2 * D, D)], wv_v, sw.at[2])
        co = pltpu.make_async_copy(wo_hbm, wo_v, sw.at[3])
        c1 = pltpu.make_async_copy(w1_hbm, w1_v, sf.at[0])
        c3 = pltpu.make_async_copy(w3_hbm, w3_v, sf.at[1])
        c2 = pltpu.make_async_copy(w2_hbm, w2_v, sf.at[2])

        def cout(t):
            r = pl.ds(pl.multiple_of(t * TM, TM), TM)
            return pltpu.make_async_copy(ob_v.at[r], o_hbm.at[r], so.at[t])

        ck.start()
        cx(0).start()
        T_v[...] = jnp.zeros_like(T_v)
        z_v[...] = jnp.zeros_like(z_v)
        ck.wait()
        cx(1).start(); cv.start(); co.start(); cq.start()
        for i in range(2, NK):
            cx(i).start()
        c1.start(); c3.start(); c2.start()

        def kbody(i, c):
            cx(i).wait()
            xi = x_v[pl.ds(pl.multiple_of(i * TK, TK), TK), :]
            pk = _phi(jnp.dot(xi, wk_v[...], preferred_element_type=_F32))
            z_v[...] += jnp.sum(pk.reshape(TK // 8, 8, D), axis=0)
            T_v[...] += lax.dot_general(pk.astype(_BF16), xi, _TN, preferred_element_type=_F32)
            return c
        lax.fori_loop(0, NK, kbody, 0)

        cv.wait(); co.wait()
        r = lax.broadcasted_iota(jnp.int32, (128, 128), 0) // _HEAD
        cc = lax.broadcasted_iota(jnp.int32, (128, 128), 1) // _HEAD
        mask = r == cc
        for g in range(NG):
            sl = pl.ds(g * 128, 128)
            kv = jnp.dot(T_v[sl, :].astype(_BF16), wv_v[:, sl], preferred_element_type=_F32)
            kv = jnp.where(mask, kv, 0.0).astype(_BF16)
            M_v[sl, :] = jnp.dot(kv, wo_v[sl, :], preferred_element_type=_F32).astype(_BF16)
            zr = jnp.sum(z_v[:, sl], axis=0, keepdims=True)
            zb_v[sl, :] = jnp.where(mask, jnp.broadcast_to(zr, (128, 128)), 0.0).astype(_BF16)

        cq.wait(); c1.wait(); c3.wait(); c2.wait()

        gw = gw_ref[...].astype(_F32).reshape(1, D)

        def tile(t, carry):
            row = pl.ds(pl.multiple_of(t * TM, TM), TM)
            xt = x_v[row, :]
            g = jax.nn.sigmoid(jnp.sum(xt.astype(_F32) * gw, axis=1, keepdims=True))
            acc = None
            for c in range(NF):
                cs = pl.ds(c * FC, FC)
                ga = jnp.dot(xt, w1_v[:, cs], preferred_element_type=_F32)
                up = jnp.dot(xt, w3_v[:, cs], preferred_element_type=_F32)
                h = (ga * jax.nn.sigmoid(ga) * up).astype(_BF16)
                d = jnp.dot(h, w2_v[cs, :], preferred_element_type=_F32)
                acc = d if acc is None else acc + d
            pq = _phi(jnp.dot(xt, wq_v[...], preferred_element_type=_F32))
            pqb = pq.astype(_BF16)
            outs = []
            for gi in range(NG):
                sl = slice(gi * 128, (gi + 1) * 128)
                den = lax.dot_general(pqb[:, sl], zb_v[pl.ds(gi * 128, 128), :], _NT,
                                      preferred_element_type=_F32) + 1e-6
                outs.append((pq[:, sl] * (g * _recip(den))).astype(_BF16))
            lhs = jnp.concatenate(outs, axis=1)
            acc = acc * (1.0 - g) + jnp.dot(lhs, M_v[...], preferred_element_type=_F32)
            ob_v[row, :] = acc.astype(_BF16)
            cout(t).start()
            return carry
        lax.fori_loop(0, NT, tile, 0)
        for t in range(NT):
            cout(t).wait()

    any_spec = pl.BlockSpec(memory_space=pl.ANY)
    out = pl.pallas_call(
        kernel,
        out_shape=jax.ShapeDtypeStruct((S, D), _BF16),
        in_specs=[any_spec] * 6 + [pl.BlockSpec(memory_space=pltpu.VMEM)],
        out_specs=any_spec,
        scratch_shapes=[
            pltpu.VMEM((S, D), _BF16),
            pltpu.VMEM((D, D), _BF16), pltpu.VMEM((D, D), _BF16), pltpu.VMEM((D, D), _BF16),
            pltpu.VMEM((D, D), _BF16),
            pltpu.VMEM((D, F), _BF16), pltpu.VMEM((D, F), _BF16), pltpu.VMEM((F, D), _BF16),
            pltpu.VMEM((D, D), _F32), pltpu.VMEM((8, D), _F32), pltpu.VMEM((D, D), _BF16),
            pltpu.VMEM((D, 128), _BF16),
            pltpu.VMEM((S, D), _BF16),
            pltpu.SemaphoreType.DMA((NK,)), pltpu.SemaphoreType.DMA((4,)),
            pltpu.SemaphoreType.DMA((3,)), pltpu.SemaphoreType.DMA((NT,)),
        ],
        compiler_params=pltpu.CompilerParams(vmem_limit_bytes=110 * 1024 * 1024),
    )(A_x.reshape(S, D), A_wqkv, A_wo, B_w1, B_w3, B_w2, gate_w)
    return out.reshape(B, S, D)
```

```python
import jax
import jax.numpy as jnp
from jax import lax
import jax.experimental.pallas as pl
import jax.experimental.pallas.tpu as pltpu

_F32, _BF16 = jnp.float32, jnp.bfloat16
_NT = (((1,), (1,)), ((), ()))
_TN = (((0,), (0,)), ((), ()))
_H = 32

_TOK = 256
_FC = 896
_WK_UNIT = 256
_WK_STEPS = (1, 1, 2)
_OSPLIT = 4


def _phi(t):
    return jnp.where(t > 0, t + 1.0, jnp.exp(t)) + 1e-6


@jax.jit
def pallas_gated_mix__linear_attn_block__glu_gated_swiglu__prompt_kernel(
    A_x: jax.Array,
    A_wqkv: jax.Array,
    A_wo: jax.Array,
    B_x: jax.Array,
    B_w1: jax.Array,
    B_w3: jax.Array,
    B_w2: jax.Array,
    gate_w: jax.Array,
):
    del B_x
    B, S, D = A_x.shape
    F = B_w1.shape[1]
    DH = D // _H
    TOK, FC, CU = _TOK, _FC, _WK_UNIT
    NT, NF, NG, NU, OW = S // TOK, F // FC, D // 128, D // CU, D // _OSPLIT
    assert B == 1 and S % TOK == 0 and F % FC == 0 and 128 % DH == 0
    assert sum(_WK_STEPS) == NU and TOK % 128 == 0
    step_off = [CU * sum(_WK_STEPS[:j]) for j in range(len(_WK_STEPS))]
    step_w = [CU * n for n in _WK_STEPS]

    def kernel(x_hbm, wqkv_hbm, wo_hbm, w1_hbm, w3_hbm, w2_hbm, gw_hbm, o_hbm,
               x_v, wq_v, wk_v, wv_v, wqT_v, wo_v, w1_v, w3_v, w2_v,
               T_v, z_v, M_v, zr_v, ob_v, gw_v, sem_x, sem_k, sem):
        sem_a, sem_f, sem_o = sem.at[0], sem.at[1], sem.at[2]

        def cp_x(i):
            r = pl.ds(pl.multiple_of(i * TOK, TOK), TOK)
            return pltpu.make_async_copy(x_hbm.at[r], x_v.at[r], sem_x.at[i])

        def cp_k(u):
            o = pl.multiple_of(u * CU, CU)
            return pltpu.make_async_copy(
                wqkv_hbm.at[:, pl.ds(D + o, CU)], wk_v.at[:, pl.ds(o, CU)], sem_k.at[u])

        def cp_out(t, s):
            r, c = pl.ds(pl.multiple_of(t * TOK, TOK), TOK), pl.ds(s * OW, OW)
            return pltpu.make_async_copy(ob_v.at[r, c], o_hbm.at[r, c], sem_o)

        attn_copies = (
            pltpu.make_async_copy(gw_hbm, gw_v, sem_a),
            pltpu.make_async_copy(wqkv_hbm.at[:, pl.ds(2 * D, D)], wv_v, sem_a),
            pltpu.make_async_copy(wo_hbm, wo_v, sem_a),
            pltpu.make_async_copy(wqkv_hbm.at[:, pl.ds(0, D)], wq_v, sem_a),
        )
        ffn_copies = (
            pltpu.make_async_copy(w1_hbm, w1_v, sem_f),
            pltpu.make_async_copy(w3_hbm, w3_v, sem_f),
            pltpu.make_async_copy(w2_hbm, w2_v, sem_f),
        )

        def start_in_order(lo, hi, make_copy):
            def body(i, carry):
                make_copy(i).start()
                return carry
            lax.fori_loop(lo, hi, body, 0)

        cp_x(0).start()
        start_in_order(0, NU, cp_k)
        start_in_order(1, NT, cp_x)
        for c in attn_copies + ffn_copies:
            c.start()

        cp_x(0).wait()
        x0 = x_v[0:TOK, :]

        def summarize_step(j, pk):
            cs = pl.ds(step_off[j], step_w[j])
            z_v[:, cs] = jnp.sum(pk.reshape(TOK // 8, 8, step_w[j]), axis=0)
            T_v[cs, :] = lax.dot_general(pk.astype(_BF16), x0, _TN, preferred_element_type=_F32)

        prev = None
        for j in range(len(_WK_STEPS)):
            for u in range(step_off[j] // CU, (step_off[j] + step_w[j]) // CU):
                cp_k(u).wait()
            pk = _phi(jnp.dot(x0, wk_v[:, pl.ds(step_off[j], step_w[j])],
                              preferred_element_type=_F32))
            if prev is not None:
                summarize_step(j - 1, prev)
            prev = pk
        summarize_step(len(_WK_STEPS) - 1, prev)

        def k_tile(i, carry):
            cp_x(i).wait()
            xi = x_v[pl.ds(pl.multiple_of(i * TOK, TOK), TOK), :]
            pk = _phi(jnp.dot(xi, wk_v[...], preferred_element_type=_F32))
            z_v[...] += jnp.sum(pk.reshape(TOK // 8, 8, D), axis=0)
            T_v[...] += lax.dot_general(pk.astype(_BF16), xi, _TN, preferred_element_type=_F32)
            return carry

        lax.fori_loop(1, NT, k_tile, 0)

        for c in attn_copies:
            c.wait()
        same_head = (lax.broadcasted_iota(jnp.int32, (128, 128), 0) // DH
                     == lax.broadcasted_iota(jnp.int32, (128, 128), 1) // DH)

        def kv_group(g):
            sl = pl.ds(g * 128, 128)
            kv = jnp.dot(T_v[sl, :].astype(_BF16), wv_v[:, sl], preferred_element_type=_F32)
            return jnp.where(same_head, kv, 0.0).astype(_BF16)

        def m_group(g, kv):
            sl = pl.ds(g * 128, 128)
            M_v[sl, :] = jnp.dot(kv, wo_v[sl, :], preferred_element_type=_F32).astype(_BF16)
            z_row = jnp.sum(z_v[:, sl], axis=0, keepdims=True)
            zr_v[sl, :] = jnp.broadcast_to(z_row, (128, 128)).T
            wqT_v[sl, :] = wq_v[:, sl].T

        kv_prev = kv_group(0)
        for g in range(1, NG):
            kv_next = kv_group(g)
            m_group(g - 1, kv_prev)
            kv_prev = kv_next
        m_group(NG - 1, kv_prev)

        for c in ffn_copies:
            c.wait()
        gw = gw_v[...].astype(_F32).reshape(1, D)

        def tile(t, carry):
            row = pl.ds(pl.multiple_of(t * TOK, TOK), TOK)
            xt = x_v[row, :]
            g = jax.nn.sigmoid(jnp.sum(xt.astype(_F32) * gw, axis=1, keepdims=True))

            acc = None
            qT = None
            for c in range(NF):
                cs = pl.ds(c * FC, FC)
                gate = jnp.dot(xt, w1_v[:, cs], preferred_element_type=_F32)
                up = jnp.dot(xt, w3_v[:, cs], preferred_element_type=_F32)
                h = gate * jax.nn.sigmoid(gate) * up
                d = jnp.dot(h.astype(_BF16), w2_v[cs, :], preferred_element_type=_F32)
                acc = d if acc is None else acc + d
                if c == 0:
                    qT = lax.dot_general(wqT_v[...], xt, _NT, preferred_element_type=_F32)

            pq = _phi(qT)
            zr = zr_v[...]
            pqz = jnp.concatenate(
                [pq[:, j * 128:(j + 1) * 128] * zr for j in range(TOK // 128)], axis=1)
            den = jnp.sum(pqz.reshape(_H, DH, TOK), axis=1, keepdims=True) + 1e-6
            lhsT = (pq.reshape(_H, DH, TOK) * (1.0 / den)).reshape(D, TOK).astype(_BF16)

            for s in range(_OSPLIT):
                cs = pl.ds(s * OW, OW)
                attn = lax.dot_general(lhsT, M_v[:, cs], _TN, preferred_element_type=_F32)
                out = acc[:, s * OW:(s + 1) * OW] * (1.0 - g) + attn * g
                ob_v[row, cs] = out.astype(_BF16)
                cp_out(t, s).start()
            return carry

        lax.fori_loop(0, NT, tile, 0)
        pltpu.make_async_copy(ob_v, o_hbm, sem_o).wait()

    hbm = pl.BlockSpec(memory_space=pl.ANY)
    out = pl.pallas_call(
        kernel,
        out_shape=jax.ShapeDtypeStruct((S, D), _BF16),
        in_specs=[hbm] * 7,
        out_specs=hbm,
        scratch_shapes=[
            pltpu.VMEM((S, D), _BF16),
            pltpu.VMEM((D, D), _BF16),
            pltpu.VMEM((D, D), _BF16),
            pltpu.VMEM((D, D), _BF16),
            pltpu.VMEM((D, D), _BF16),
            pltpu.VMEM((D, D), _BF16),
            pltpu.VMEM((D, F), _BF16),
            pltpu.VMEM((D, F), _BF16),
            pltpu.VMEM((F, D), _BF16),
            pltpu.VMEM((D, D), _F32),
            pltpu.VMEM((8, D), _F32),
            pltpu.VMEM((D, D), _BF16),
            pltpu.VMEM((D, 128), _F32),
            pltpu.VMEM((S, D), _BF16),
            pltpu.VMEM((D,), _BF16),
            pltpu.SemaphoreType.DMA((NT,)),
            pltpu.SemaphoreType.DMA((NU,)),
            pltpu.SemaphoreType.DMA((3,)),
        ],
        compiler_params=pltpu.CompilerParams(vmem_limit_bytes=100 * 1024 * 1024),
    )(A_x.reshape(S, D), A_wqkv, A_wo, B_w1, B_w3, B_w2, gate_w)
    return out.reshape(B, S, D)
```
